```python
import os as _os
_os.environ.setdefault('JAX_PLATFORMS', 'cpu')
import jax
import jax.numpy as jnp

def _softmax(x, axis=-1):
    return jax.nn.softmax(x, axis=axis)

def _gelu(x):
    return jax.nn.gelu(x, approximate=True)

def _silu(x):
    return jax.nn.silu(x)

def _sigmoid(x):
    return jax.nn.sigmoid(x)

def _layernorm(x, axis=-1, eps=1e-05):
    m = jnp.mean(x, axis=axis, keepdims=True)
    v = jnp.var(x, axis=axis, keepdims=True)
    return (x - m) / jnp.sqrt(v + eps)

def _scatter_add(tgt, idx, src, axis=0):
    return tgt.at[idx].add(src)

def _segment_sum(src, seg, n):
    return jax.ops.segment_sum(src, seg, n)

class _Rng:

    def __init__(self, key):
        self._k = key

    def _next(self):
        self._k, sub = jax.random.split(self._k)
        return sub

    def normal(self, shape):
        return jax.random.normal(self._next(), shape, dtype=jnp.bfloat16)

    def randint(self, lo, hi, shape):
        return jax.random.randint(self._next(), shape, lo, hi, dtype=jnp.int32)

    def uniform(self, shape, lo=0.0, hi=1.0):
        return jax.random.uniform(self._next(), shape, jnp.bfloat16, lo, hi)

    def permutation(self, n):
        return jax.random.permutation(self._next(), n)
kernel_name = 'adaLN_cond__sliding_local_dilated__dense_activation_relu__prompt'

def setup_inputs():
    _rng = _Rng(jax.random.key(int.from_bytes(__import__("os").urandom(4), "little")))
    _w = lambda a: (lambda t: t.astype(jnp.bfloat16) if jnp.issubdtype(t.dtype, jnp.floating) else t)(jnp.asarray(a))

    def _A_setup():
        B, S, D = (1, 2048, 576)
        return {'x': _w((lambda *s: _rng.normal(s) * 0.05)(B, S, D)), 'wqkv': _w((lambda *s: _rng.normal(s) * 0.05)(D, 3 * D)), 'wo': _w((lambda *s: _rng.normal(s) * 0.05)(D, D))}
    _A_in = _A_setup()

    def _B_setup():
        B, S, D, Dff = (1, 2048, 576, 4608)
        return {'x': _w((lambda *s: _rng.normal(s) * 0.05)(B, S, D)), 'w1': _w((lambda *s: _rng.normal(s) * 0.05)(D, Dff)), 'w2': _w((lambda *s: _rng.normal(s) * 0.05)(Dff, D))}
    _B_in = _B_setup()
    return {'A_x': _A_in['x'], 'A_wqkv': _A_in['wqkv'], 'A_wo': _A_in['wo'], 'B_x': _B_in['x'], 'B_w1': _B_in['w1'], 'B_w2': _B_in['w2'], 'c': _w((lambda *s: _rng.normal(s) * 0.05)(1, 576) * 8.0), 'w_mod': _w((lambda *s: _rng.normal(s) * 0.05)(576, 6 * 576) * 576 ** (-0.5) * 8.0)}

def reference(A_x, A_wqkv, A_wo, B_x, B_w1, B_w2, c, w_mod):

    def _A_ref(x, wqkv, wo):
        B, S, D = x.shape
        H = 32
        Dh = D // H
        W, dil = (8, 2)
        qkv = (lambda x, *d: x.transpose(*d))((x @ wqkv).reshape(B, S, 3, H, Dh), 2, 0, 3, 1, 4)
        q, k, v = (qkv[0], qkv[1], qkv[2])
        scale = Dh ** (-0.5)
        pos = jnp.arange(S)
        off = jnp.arange(W) * dil
        idx = pos[:, None] - off[None, :]
        mask = idx >= 0
        idx_c = jnp.where(mask, idx, 0).reshape(-1)
        kg = k[:, :, idx_c, :].reshape(B, H, S, W, Dh)
        vg = v[:, :, idx_c, :].reshape(B, H, S, W, Dh)
        logits = jnp.einsum('bhsd,bhswd->bhsw', q, kg) * scale
        logits = jnp.where(mask[None, None, :, :], logits, -1000000000.0)
        attn = _softmax(logits, axis=-1)
        o = jnp.einsum('bhsw,bhswd->bhsd', attn, vg)
        return (lambda x, *d: x.transpose(*d))(o, 0, 2, 1, 3).reshape(B, S, D) @ wo

    def _B_ref(x, w1, w2):
        h = jnp.einsum('bsd,df->bsf', x, w1)
        zero = jnp.zeros_like(h)
        h = jnp.maximum(h, zero)
        return jnp.einsum('bsf,fd->bsd', h, w2)
    x = A_x
    mod = (_silu(c) @ w_mod).reshape(c.shape[0], 6, 1, -1)
    sa, ca, ga, sb, cb, gb = (mod[:, 0].copy(), mod[:, 1].copy(), mod[:, 2].copy(), mod[:, 3].copy(), mod[:, 4].copy(), mod[:, 5].copy())
    h = _layernorm(x, axis=-1) * (1 + ca) + sa
    x = x + ga * _A_ref(h, A_wqkv, A_wo)
    h = _layernorm(x, axis=-1) * (1 + cb) + sb
    x = x + gb * _B_ref(h, B_w1, B_w2)
    return x
```

```python
import numpy as np
import jax
import jax.numpy as jnp
import jax.experimental.pallas as pl
import jax.experimental.pallas.tpu as pltpu

S, D, F = 2048, 576, 4608
H, DH, W = 32, 18, 8
DP = 640
HALO = 16
TM = int(256)
RC = int('8')
FC = int(768)
NT = int(S // TM)
NF = F // FC
POSQ = int('3')
POSW = int('8')
POSA = [int(x) for x in '3'.split(',')]
PIPE = int(0)
K = int('3')
GATE = 'out'
GKIND = 'iota'
AK_GATED = int(1)
SSPLIT = int(0)
PSPLIT = int('3')
P0 = 'wc,m:0,wx:0,l:0,ww:0,pp:0,ww:1,q:0,pp:1,ww:2,wx:1,k:0,pp:2,l:1,v:0,'
PRO = P0 + 'qkv:1,a:0:32:e,wwo,wm:1,wm:2,wx:2,wx:3,wx:4,l:2,pw,m:1,m:2,qkv:2,w:0,a:1:32:e,lq:3,a:2:32:e,w:1,wf:0:4,a:3'
DMAORD = 'c,m0,x0,q0,q1,q2,x1,wo,m1,m2,x2,x3,x4,a0,b0,a1,b1,a2,b2,a3,b3,x5,x6,x7,a4,b4,a5,b5'
T0 = 'w:2|||wf:4:6,wx:5,wx:6,wx:7|w:3,lq:4,a:4|'
GDEPTH = int(1)
RCP = int(RC)
GATEP = GATE
X1S = int(K + 1)
BAR = 'sem'
WSPLIT = [int(x) for x in '3'.split(',')]
WGROUPS = list(zip([0] + WSPLIT, WSPLIT + [NF]))
SCOPES = int(0)
EPS = 1e-5
FLAGS = {k: True for k in 'XLA_TPU_FORCE_LP_LLO_SCHEDULER'.split(',') if k}
SCALE_LOG2E = float(DH ** -0.5 * np.log2(np.e))
f32 = jnp.float32
bf16 = jnp.bfloat16
NT_DIMS = (((1,), (1,)), ((), ()))
QKV_SPLITS = (0, 640, 1152, 1728)


class _Null:
    def __enter__(self):
        return self

    def __exit__(self, *a):
        return False


def scope(name):
    return jax.named_scope(name) if SCOPES else _Null()


def _kernel(xT_hbm, c_hbm, wqkv_hbm, wo_hbm, w1_hbm, w2T_hbm, wmod_hbm, outT_hbm,
            xT_s, outT_s, c_s, wqkv_raw, stage, wqkvT, wo_raw, woL, w1_s, w2T_s, wmod_s, modT,
            h_buf, qbuf, kbuf, vbuf, obuf, h2buf, x1buf, gate,
            sems, w1sems, w2sems, xsems, osems, bar_sem):

    def x_copy(t):
        return pltpu.make_async_copy(xT_hbm.at[0, :, t * TM:(t + 1) * TM], xT_s.at[:, t * TM:(t + 1) * TM], xsems.at[t])

    def out_copy(t):
        return pltpu.make_async_copy(outT_s.at[:, t * TM:(t + 1) * TM], outT_hbm.at[0, :, t * TM:(t + 1) * TM], osems.at[t])

    def cols_copy(src, dst, lo, hi, sem):
        return pltpu.make_async_copy(src.at[:, lo:hi], dst.at[:, lo:hi], sem)

    def wqkv_copy(p):
        return cols_copy(wqkv_hbm, wqkv_raw, QKV_SPLITS[p], QKV_SPLITS[p + 1], sems.at[p])

    def wmod_copy(p):
        return cols_copy(wmod_hbm, wmod_s, p * 2 * D, (p + 1) * 2 * D, sems.at[3 + p])

    def w1_copy(f):
        return cols_copy(w1_hbm, w1_s, f * FC, (f + 1) * FC, w1sems.at[f])

    def w2_copy(f):
        return cols_copy(w2T_hbm, w2T_s, f * FC, (f + 1) * FC, w2sems.at[f])

    def c_copy():
        return pltpu.make_async_copy(c_hbm, c_s, sems.at[6])

    def wo_copy():
        return pltpu.make_async_copy(wo_hbm, wo_raw, sems.at[7])

    dma = {'c': c_copy, 'wo': wo_copy}
    dma.update({f'm{p}': (lambda p=p: wmod_copy(p)) for p in range(3)})
    dma.update({f'q{p}': (lambda p=p: wqkv_copy(p)) for p in range(3)})
    dma.update({f'x{t}': (lambda t=t: x_copy(t)) for t in range(NT)})
    dma.update({f'a{f}': (lambda f=f: w1_copy(f)) for f in range(NF)})
    dma.update({f'b{f}': (lambda f=f: w2_copy(f)) for f in range(NF)})
    order = [dma.pop(k) for k in DMAORD.split(',') if k in dma]
    assert not dma, dma
    for mk in order:
        if BAR == 'when':
            pl.when(pl.program_id(0) == 0)(lambda mk=mk: mk().start())
        elif BAR == 'sem':
            mk().start()
            pl.semaphore_signal(bar_sem, 1)
            pl.semaphore_wait(bar_sem, 1)
        elif BAR == 'delay':
            mk().start()
            pl.delay(0)
        else:
            mk().start()

    kbuf[:, 0:HALO, :] = jnp.zeros((5, HALO, 128), f32)
    vbuf[:, 0:HALO, :] = jnp.zeros((5, HALO, 128), f32)
    gate[...] = jnp.zeros((RC, 128), f32)
    dep = {}
    h_buf[:, :, D:DP] = jnp.zeros((2, TM, DP - D), bf16)

    def st_mod(p):
        cv = c_s[...].astype(f32)
        sc = jnp.broadcast_to((cv * jax.nn.sigmoid(cv)).astype(bf16), (8, D))
        for t in range(2 * D // 128):
            lo = p * 2 * D + t * 128
            m = jnp.dot(sc, wmod_s[:, lo:lo + 128], preferred_element_type=f32)
            mt = jnp.broadcast_to(m[0:1, :], (128, 128)).astype(bf16).T.astype(f32)
            row = lo + jax.lax.broadcasted_iota(jnp.int32, (128, 128), 0)
            if (lo < 2 * D and lo + 128 > D) or (lo < 5 * D and lo + 128 > 4 * D):
                is_scale = ((row >= D) & (row < 2 * D)) | ((row >= 4 * D) & (row < 5 * D))
                mt = mt + jnp.where(is_scale, 1.0, 0.0)
            modT[lo:lo + 128, :] = mt

    def st_prep_w(p):
        lo = (p * D // 128) * 128
        off = p * D - lo
        wd = min(640, 3 * D - lo)
        for t in range(5):
            kd = min(128, D - t * 128)
            blk = wqkv_raw[t * 128:t * 128 + kd, lo:lo + wd]
            if kd < 128:
                blk = jnp.concatenate([blk, jnp.zeros((128 - kd, wd), bf16)], axis=0)
            stage[t, 0:wd, :] = blk.T.astype(f32)
            for d in range(DH):
                rows = stage[t, pl.ds(off + d, H, stride=DH), :]
                r0 = p * 512 + d * H if d < 16 else 1536 + p * 64 + (d - 16) * H
                wqkvT[r0:r0 + H, t * 128:(t + 1) * 128] = rows.astype(bf16)
            if p == 2:
                wqkvT[1728:1792, t * 128:(t + 1) * 128] = jnp.zeros((64, 128), bf16)

    def st_prep_wo():
        for t in range(5):
            wd = min(128, D - t * 128)
            blk = wo_raw[:, t * 128:t * 128 + wd].astype(f32)
            if wd < 128:
                blk = jnp.concatenate([blk, jnp.zeros((D, 128 - wd), f32)], axis=1)
            stage[t, 0:D, :] = blk
            parts = [stage[t, pl.ds(d, H, stride=DH), :].astype(bf16) for d in range(DH)]
            parts.append(jnp.zeros((DP - D, 128), bf16))
            wop = jnp.concatenate(parts, axis=0)
            woL[t * 128:t * 128 + wd, :] = wop.T[0:wd, :]

    def ln_mod_col(x, r_shift, r_scale):
        mean = jnp.mean(x, axis=0, keepdims=True)
        xc = x - mean
        var = jnp.mean(xc * xc, axis=0, keepdims=True)
        y = xc * jax.lax.rsqrt(var + EPS)
        return (y * modT[r_scale * D:(r_scale + 1) * D, :] + modT[r_shift * D:(r_shift + 1) * D, :]).astype(bf16)

    def st_ln1(t):
        for j in range(TM // 128):
            x = xT_s[:, t * TM + j * 128:t * TM + (j + 1) * 128].astype(f32)
            h_buf[t % 2, j * 128:(j + 1) * 128, 0:D] = ln_mod_col(x, 0, 1).T

    def proj(t, lo, hi):
        return jax.lax.dot_general(h_buf[t % 2], wqkvT[lo:hi, :], NT_DIMS, preferred_element_type=f32)

    def st_q(t):
        qbuf[t % 3, :, 0:512] = proj(t, 0, 512) * SCALE_LOG2E

    def st_kv(t, p):
        r = proj(t, p * 512, (p + 1) * 512)
        buf = kbuf if p == 1 else vbuf
        rows = slice(HALO + t * TM, HALO + (t + 1) * TM)
        for j in range(4):
            buf[j, rows, :] = r[:, j * 128:(j + 1) * 128]
        if p == 1:
            qk = proj(t, 1536, 1664)
            qbuf[t % 3, :, 512:640] = qk * SCALE_LOG2E
            lane = jax.lax.broadcasted_iota(jnp.int32, (TM, 128), 1)
            kbuf[4, rows, :] = jnp.where(lane < 64, pltpu.roll(qk, 64, 1), 0.0)
        else:
            vbuf[4, rows, :] = proj(t, 1664, 1792)

    def st_attn(t, ci, RC=RC, GATE=GATE):
        r0 = ci * RC
        g0 = t * TM + r0
        q = [qbuf[t % 3, r0:r0 + RC, j * 128:(j + 1) * 128] for j in range(5)]
        if GATE and ci >= GDEPTH:
            dd = dep[(t, ci - GDEPTH)]
            never = dd > 2.0
            q = [jnp.where(never, dd, x) for x in q]
        ss = []
        for w in range(W):
            if GATE and SSPLIT and w > 0 and w % SSPLIT == 0:
                dd = ss[w - 1]
                never = dd != dd + 0.0 if False else (dd - dd) > 2.0
                q = [jnp.where(never, dd, x) for x in q]
            p = [q[j] * kbuf[j, g0 + HALO - 2 * w:g0 + HALO - 2 * w + RC, :] for j in range(5)]
            s = (p[0] + p[1]) + (p[2] + p[3]) + p[4]
            s = s + pltpu.roll(s, 64, 1)
            s = s + pltpu.roll(s, 32, 1)
            if t * TM + r0 < 2 * w:
                row = t * TM + r0 + jax.lax.broadcasted_iota(jnp.int32, (RC, 128), 0)
                s = jnp.where(row >= 2 * w, s, -1e30)
            ss.append(s)
        m = ss[0]
        for w in range(1, W):
            m = jnp.maximum(m, ss[w])
        es = [jnp.exp2(s - m) for s in ss]
        den = es[0]
        for w in range(1, W):
            den = den + es[w]
        inv = 1.0 / den
        if GATE == 'e':
            dep[(t, ci)] = es[W - 1]
        if GATE == 'inv':
            dep[(t, ci)] = inv * es[0]
        for j in range(5):
            acc = None
            if GATE and PSPLIT and j > 0 and j % PSPLIT == 0:
                never = prev_e > 2.0
                es = [jnp.where(never, o, e) for e in es]
            for w in range(W):
                tt = es[w] * vbuf[j, g0 + HALO - 2 * w:g0 + HALO - 2 * w + RC, :]
                acc = tt if acc is None else acc + tt
            o = acc * inv
            prev_e = es[0] + o * 0.0
            if GATE == 'out' and j == 4:
                dep[(t, ci)] = es[0] + o * 0.0
            obuf[t % 3, r0:r0 + RC, j * 128:(j + 1) * 128] = o.astype(bf16)

    def st_attn_all(t, rc=RCP, g=GATEP):
        for ci in range(TM // rc):
            st_attn(t, ci, rc, g)

    def st_wo_ln2(t):
        aT = jax.lax.dot_general(woL[...], obuf[t % 3], NT_DIMS, preferred_element_type=f32)
        for j in range(TM // 128):
            x = xT_s[:, t * TM + j * 128:t * TM + (j + 1) * 128].astype(f32)
            x1 = x + modT[2 * D:3 * D, :] * aT[:, j * 128:(j + 1) * 128]
            x1buf[t % X1S, :, j * 128:(j + 1) * 128] = x1
            h2buf[t * TM + j * 128:t * TM + (j + 1) * 128, :] = ln_mod_col(x1, 3, 4).T

    def st_m1(t, f):
        h1 = jnp.dot(h2buf[t * TM:(t + 1) * TM, :], w1_s[:, f * FC:(f + 1) * FC], preferred_element_type=f32)
        return jnp.maximum(h1, 0.0).astype(bf16)

    def st_m2(t, f, h1):
        return jax.lax.dot_general(w2T_s[:, f * FC:(f + 1) * FC], h1, NT_DIMS, preferred_element_type=f32)

    def st_out(t, acc):
        for j in range(TM // 128):
            o = x1buf[t % X1S, :, j * 128:(j + 1) * 128] + modT[5 * D:6 * D, :] * acc[:, j * 128:(j + 1) * 128]
            outT_s[:, t * TM + j * 128:t * TM + (j + 1) * 128] = o.astype(bf16)
        out_copy(t).start()

    def st_lq(t):
        st_ln1(t)
        st_q(t)
        st_kv(t, 1)
        st_kv(t, 2)

    def bar():
        wo_copy().wait()
        wmod_copy(1).wait()
        wmod_copy(2).wait()
        for t in range(2, NXE):
            x_copy(t).wait()

    def run_tokens(spec):
        for tok in spec.split(','):
            if not tok:
                continue
            name, *args = tok.split(':')
            if SCOPES and name in ('wc', 'wx', 'ww', 'wwo', 'wm', 'wf'):
                with scope('z_' + tok.replace(':', '_')):
                    run_tok(name, args, tok)
            else:
                run_tok(name, args, tok)

    def run_tok(name, args, tok):
        if True:
            if name == 'wc':
                c_copy().wait()
                wmod_copy(0).wait()
            elif name == 'wx':
                if int(args[0]) < NT:
                    x_copy(int(args[0])).wait()
            elif name == 'ww':
                wqkv_copy(int(args[0])).wait()
            elif name == 'wwo':
                wo_copy().wait()
            elif name == 'wm':
                wmod_copy(int(args[0])).wait()
            elif name == 'wf':
                for f in range(int(args[0]), int(args[1])):
                    w1_copy(f).wait()
                    w2_copy(f).wait()
            elif name == 'pp':
                st_prep_w(int(args[0]))
            elif name == 'm':
                st_mod(int(args[0]))
            elif name == 'l':
                st_ln1(int(args[0]))
            elif name == 'q':
                st_q(int(args[0]))
            elif name == 'k':
                st_kv(int(args[0]), 1)
            elif name == 'v':
                st_kv(int(args[0]), 2)
            elif name == 'lq':
                if int(args[0]) < NT:
                    st_lq(int(args[0]))
            elif name == 'qkv':
                st_q(int(args[0]))
                st_kv(int(args[0]), 1)
                st_kv(int(args[0]), 2)
            elif name == 'a':
                if int(args[0]) < NT:
                    if len(args) > 1:
                        st_attn_all(int(args[0]), int(args[1]), args[2])
                    else:
                        st_attn_all(int(args[0]), RC, GATE)
            elif name == 'w':
                if int(args[0]) < NT:
                    st_wo_ln2(int(args[0]))
            elif name == 'pw':
                st_prep_wo()
            else:
                raise ValueError(tok)

    run_tokens(PRO)

    events = {}
    for u in range(K + 1, NT):
        g0 = (u - K - 1) * NF
        if u > K + 1:
            events.setdefault(g0 + POSQ, []).append(f"lq:{u},a:{u}")
        events.setdefault(g0 + POSW, []).append(f"w:{u}")
    t0 = T0.split('|')

    pending = None
    for t in range(NT):
        with scope(f"tile{t}"):
            acc = None
            for f in range(NF):
                r = st_m2(t, f, st_m1(t, f))
                acc = r if acc is None else acc + r
                if f == 0 and pending is not None:
                    st_out(*pending)
                if t == 0:
                    run_tokens(t0[f])
                for spec in events.get(t * NF + f, []):
                    run_tokens(spec)
            pending = (t, acc)
    with scope("tail"):
        st_out(*pending)
        for t in range(NT):
            out_copy(t).wait()


@jax.jit
def pallas_adaLN_cond__sliding_local_dilated__dense_activation_relu__prompt_kernel(
        A_x, A_wqkv, A_wo, B_x, B_w1, B_w2, c, w_mod):
    del B_x
    hbm = pl.BlockSpec(memory_space=pltpu.HBM)
    xT = jnp.transpose(A_x, (0, 2, 1))
    w2T = jnp.transpose(B_w2)
    outT = pl.pallas_call(
        _kernel,
        grid=(1,),
        in_specs=[hbm] * 7,
        out_specs=hbm,
        out_shape=jax.ShapeDtypeStruct((1, D, S), A_x.dtype),
        scratch_shapes=[
            pltpu.VMEM((D, S), bf16),
            pltpu.VMEM((D, S), bf16),
            pltpu.VMEM((1, D), bf16),
            pltpu.VMEM((D, 3 * D), bf16),
            pltpu.VMEM((5, DP, 128), f32),
            pltpu.VMEM((1792, DP), bf16),
            pltpu.VMEM((D, D), bf16),
            pltpu.VMEM((D, DP), bf16),
            pltpu.VMEM((D, F), bf16),
            pltpu.VMEM((D, F), bf16),
            pltpu.VMEM((D, 6 * D), bf16),
            pltpu.VMEM((6 * D, 128), f32),
            pltpu.VMEM((2, TM, DP), bf16),
            pltpu.VMEM((3, TM, DP), f32),
            pltpu.VMEM((5, HALO + S, 128), f32),
            pltpu.VMEM((5, HALO + S, 128), f32),
            pltpu.VMEM((3, TM, DP), bf16),
            pltpu.VMEM((S, D), bf16),
            pltpu.VMEM((X1S, D, TM), f32),
            pltpu.VMEM((RC, 128), f32),
            pltpu.SemaphoreType.DMA((8,)),
            pltpu.SemaphoreType.DMA((NF,)),
            pltpu.SemaphoreType.DMA((NF,)),
            pltpu.SemaphoreType.DMA((NT,)),
            pltpu.SemaphoreType.DMA((NT,)),
            pltpu.SemaphoreType.REGULAR,
        ],
        compiler_params=pltpu.CompilerParams(vmem_limit_bytes=100 * 1024 * 1024, flags=FLAGS),
        name="adaln_block",
    )(xT, c, A_wqkv, A_wo, B_w1, w2T, w_mod)
    return jnp.transpose(outT, (0, 2, 1))
```

```python
import numpy as np
import jax
import jax.numpy as jnp
import jax.experimental.pallas as pl
import jax.experimental.pallas.tpu as pltpu

S, D, F = 2048, 576, 4608
H, DH, W = 32, 18, 8
DP = 640
HALO = 16
TM = 256
FC = 768
NT, NF = S // TM, F // FC
NQKV = 1792
QKV_SPLITS = (0, 640, 1152, 1728)
EPS = 1e-5
SCALE_LOG2E = float(DH ** -0.5 * np.log2(np.e))
NT_DIMS = (((1,), (1,)), ((), ()))
f32 = jnp.float32
bf16 = jnp.bfloat16


def _kernel(xT_hbm, c_hbm, wqkv_hbm, wo_hbm, w1_hbm, w2T_hbm, wmod_hbm, outT_hbm,
            xT_s, outT_s, c_s, wqkv_raw, stage, wqkvT, wo_raw, woL, w1_s, w2T_s, wmod_s, modT,
            h_buf, qbuf, kbuf, vbuf, obuf, h2buf, x1buf,
            sems, w1sems, w2sems, xsems, osems, order_sem):

    def cols_copy(src, dst, lo, hi, sem):
        return pltpu.make_async_copy(src.at[:, lo:hi], dst.at[:, lo:hi], sem)

    def x_copy(t):
        cols = slice(t * TM, (t + 1) * TM)
        return pltpu.make_async_copy(xT_hbm.at[0, :, cols], xT_s.at[:, cols], xsems.at[t])

    def out_copy(lo, hi, s):
        return pltpu.make_async_copy(outT_s.at[:, lo:hi], outT_hbm.at[0, :, lo:hi], osems.at[s])

    out_parts = [(t * TM, (t + 1) * TM) for t in range(NT - 1)]
    out_parts += [((NT - 1) * TM + j * 128, (NT - 1) * TM + (j + 1) * 128) for j in range(TM // 128)]

    def wqkv_copy(p):
        return cols_copy(wqkv_hbm, wqkv_raw, QKV_SPLITS[p], QKV_SPLITS[p + 1], sems.at[p])

    def wmod_copy(p):
        return cols_copy(wmod_hbm, wmod_s, p * 2 * D, (p + 1) * 2 * D, sems.at[3 + p])

    def c_copy():
        return pltpu.make_async_copy(c_hbm, c_s, sems.at[6])

    def wo_copy():
        return pltpu.make_async_copy(wo_hbm, wo_raw, sems.at[7])

    def w1_copy(f):
        return cols_copy(w1_hbm, w1_s, f * FC, (f + 1) * FC, w1sems.at[f])

    def w2_copy(f):
        return cols_copy(w2T_hbm, w2T_s, f * FC, (f + 1) * FC, w2sems.at[f])

    loads = [c_copy(), wmod_copy(0), wqkv_copy(0), x_copy(0), wqkv_copy(1), wqkv_copy(2),
             x_copy(1), x_copy(2), wo_copy(), wmod_copy(1), wmod_copy(2), x_copy(3), x_copy(4)]
    for f in range(4):
        loads += [w1_copy(f), w2_copy(f)]
    loads += [x_copy(t) for t in range(5, NT)]
    for f in range(4, NF):
        loads += [w1_copy(f), w2_copy(f)]
    for cp in loads:
        cp.start()
        pl.semaphore_signal(order_sem, 1)
        pl.semaphore_wait(order_sem, 1)

    kbuf[:, 0:HALO, :] = jnp.zeros((5, HALO, 128), f32)
    vbuf[:, 0:HALO, :] = jnp.zeros((5, HALO, 128), f32)
    h_buf[:, :, D:DP] = jnp.zeros((2, TM, DP - D), bf16)

    def st_mod(p):
        cv = c_s[...].astype(f32)
        sc = jnp.broadcast_to((cv * jax.nn.sigmoid(cv)).astype(bf16), (8, D))
        for t in range(2 * D // 128):
            lo = p * 2 * D + t * 128
            m = jnp.dot(sc, wmod_s[:, lo:lo + 128], preferred_element_type=f32)
            mt = jnp.broadcast_to(m[0:1, :], (128, 128)).astype(bf16).T.astype(f32)
            if (lo < 2 * D and lo + 128 > D) or (lo < 5 * D and lo + 128 > 4 * D):
                row = lo + jax.lax.broadcasted_iota(jnp.int32, (128, 128), 0)
                is_scale = ((row >= D) & (row < 2 * D)) | ((row >= 4 * D) & (row < 5 * D))
                mt = mt + jnp.where(is_scale, 1.0, 0.0)
            modT[lo:lo + 128, :] = mt

    def mod(r):
        return modT[r * D:(r + 1) * D, :]

    def st_prep_w(p):
        lo = (p * D // 128) * 128
        off = p * D - lo
        wd = min(640, 3 * D - lo)
        for t in range(5):
            kd = min(128, D - t * 128)
            blk = wqkv_raw[t * 128:t * 128 + kd, lo:lo + wd]
            if kd < 128:
                blk = jnp.concatenate([blk, jnp.zeros((128 - kd, wd), bf16)], axis=0)
            stage[t, 0:wd, :] = blk.T.astype(f32)
            for d in range(DH):
                rows = stage[t, pl.ds(off + d, H, stride=DH), :]
                r0 = p * 512 + d * H if d < 16 else 1536 + p * 64 + (d - 16) * H
                wqkvT[r0:r0 + H, t * 128:(t + 1) * 128] = rows.astype(bf16)
            if p == 2:
                wqkvT[1728:NQKV, t * 128:(t + 1) * 128] = jnp.zeros((NQKV - 1728, 128), bf16)

    def st_prep_wo():
        for t in range(5):
            wd = min(128, D - t * 128)
            blk = wo_raw[:, t * 128:t * 128 + wd].astype(f32)
            if wd < 128:
                blk = jnp.concatenate([blk, jnp.zeros((D, 128 - wd), f32)], axis=1)
            stage[t, 0:D, :] = blk
            parts = [stage[t, pl.ds(d, H, stride=DH), :].astype(bf16) for d in range(DH)]
            parts.append(jnp.zeros((DP - D, 128), bf16))
            woL[t * 128:t * 128 + wd, :] = jnp.concatenate(parts, axis=0).T[0:wd, :]

    def x_col(t, j):
        return xT_s[:, t * TM + j * 128:t * TM + (j + 1) * 128].astype(f32)

    def ln_mod(x, r_shift, r_scale):
        mean = jnp.mean(x, axis=0, keepdims=True)
        xc = x - mean
        var = jnp.mean(xc * xc, axis=0, keepdims=True)
        y = xc * jax.lax.rsqrt(var + EPS)
        return (y * mod(r_scale) + mod(r_shift)).astype(bf16).T

    def st_ln1(t):
        for j in range(TM // 128):
            h_buf[t % 2, j * 128:(j + 1) * 128, 0:D] = ln_mod(x_col(t, j), 0, 1)

    def proj(t, lo, hi):
        return jax.lax.dot_general(h_buf[t % 2], wqkvT[lo:hi, :], NT_DIMS, preferred_element_type=f32)

    def st_q(t):
        qbuf[t % 3, :, 0:512] = proj(t, 0, 512) * SCALE_LOG2E

    def st_kv(t, p):
        r = proj(t, p * 512, (p + 1) * 512)
        buf = kbuf if p == 1 else vbuf
        rows = slice(HALO + t * TM, HALO + (t + 1) * TM)
        for j in range(4):
            buf[j, rows, :] = r[:, j * 128:(j + 1) * 128]
        if p == 1:
            qk = proj(t, 1536, 1664)
            qbuf[t % 3, :, 512:640] = qk * SCALE_LOG2E
            lane = jax.lax.broadcasted_iota(jnp.int32, (TM, 128), 1)
            kbuf[4, rows, :] = jnp.where(lane < 64, pltpu.roll(qk, 64, 1), 0.0)
        else:
            vbuf[4, rows, :] = proj(t, 1664, NQKV)

    def st_qkv(t):
        st_q(t)
        st_kv(t, 1)
        st_kv(t, 2)

    def st_attn(t, rc, chain_on_output):
        prev = None
        for r0 in range(0, TM, rc):
            g0 = t * TM + r0
            q = [qbuf[t % 3, r0:r0 + rc, j * 128:(j + 1) * 128] for j in range(5)]
            if prev is not None:
                never = prev > 2.0
                q = [jnp.where(never, prev, x) for x in q]
            ss = []
            for w in range(W):
                rows = slice(g0 + HALO - 2 * w, g0 + HALO - 2 * w + rc)
                p = [q[j] * kbuf[j, rows, :] for j in range(5)]
                s = (p[0] + p[1]) + (p[2] + p[3]) + p[4]
                s = s + pltpu.roll(s, 64, 1)
                s = s + pltpu.roll(s, 32, 1)
                if g0 < 2 * w:
                    row = g0 + jax.lax.broadcasted_iota(jnp.int32, (rc, 128), 0)
                    s = jnp.where(row >= 2 * w, s, -1e30)
                ss.append(s)
            m = ss[0]
            for w in range(1, W):
                m = jnp.maximum(m, ss[w])
            es = [jnp.exp2(s - m) for s in ss]
            den = es[0]
            for w in range(1, W):
                den = den + es[w]
            inv = 1.0 / den
            prev = es[W - 1]
            for j in range(5):
                if j > 0 and j % 2 == 0:
                    never = tail > 2.0
                    es = [jnp.where(never, o, e) for e in es]
                acc = None
                for w in range(W):
                    rows = slice(g0 + HALO - 2 * w, g0 + HALO - 2 * w + rc)
                    tt = es[w] * vbuf[j, rows, :]
                    acc = tt if acc is None else acc + tt
                o = acc * inv
                tail = es[0] + o * 0.0
                obuf[t % 3, r0:r0 + rc, j * 128:(j + 1) * 128] = o.astype(bf16)
            if chain_on_output:
                prev = tail

    def st_wo_ln2(t):
        aT = jax.lax.dot_general(woL[...], obuf[t % 3], NT_DIMS, preferred_element_type=f32)
        for j in range(TM // 128):
            x1 = x_col(t, j) + mod(2) * aT[:, j * 128:(j + 1) * 128]
            x1buf[t % 4, :, j * 128:(j + 1) * 128] = x1
            h2buf[t * TM + j * 128:t * TM + (j + 1) * 128, :] = ln_mod(x1, 3, 4)

    def st_ffn(t, f):
        cols = slice(f * FC, (f + 1) * FC)
        h1 = jnp.dot(h2buf[t * TM:(t + 1) * TM, :], w1_s[:, cols], preferred_element_type=f32)
        h1 = jnp.maximum(h1, 0.0).astype(bf16)
        return jax.lax.dot_general(w2T_s[:, cols], h1, NT_DIMS, preferred_element_type=f32)

    def st_out(t, acc):
        for j in range(TM // 128):
            o = x1buf[t % 4, :, j * 128:(j + 1) * 128] + mod(5) * acc[:, j * 128:(j + 1) * 128]
            outT_s[:, t * TM + j * 128:t * TM + (j + 1) * 128] = o.astype(bf16)
            if t == NT - 1:
                out_copy(*out_parts[t + j], t + j).start()
        if t < NT - 1:
            out_copy(*out_parts[t], t).start()

    c_copy().wait()
    wmod_copy(0).wait()
    st_mod(0)
    wqkv_copy(0).wait()
    st_prep_w(0)
    x_copy(0).wait()
    st_ln1(0)
    wqkv_copy(1).wait()
    st_q(0)
    st_prep_w(1)
    wqkv_copy(2).wait()
    st_kv(0, 1)
    st_prep_w(2)
    x_copy(1).wait()
    x_copy(2).wait()
    st_kv(0, 2)
    st_ln1(1)
    st_qkv(1)
    st_attn(0, 16, False)
    st_ln1(2)
    wo_copy().wait()
    wmod_copy(1).wait()
    wmod_copy(2).wait()
    x_copy(3).wait()
    x_copy(4).wait()
    st_qkv(2)
    st_attn(1, 16, False)
    st_prep_wo()
    st_mod(1)
    st_mod(2)
    st_wo_ln2(0)
    st_ln1(3)
    st_qkv(3)
    st_attn(2, 16, False)
    for f in range(4):
        w1_copy(f).wait()
        w2_copy(f).wait()
    st_attn(3, 8, True)

    pending = None
    for t in range(NT):
        acc = None
        for f in range(NF):
            r = st_ffn(t, f)
            acc = r if acc is None else acc + r
            if f == 0 and pending is not None:
                st_out(*pending)
            if t == 0:
                if f == 0:
                    st_wo_ln2(1)
                    st_wo_ln2(2)
                elif f == 3:
                    for g in range(4, NF):
                        w1_copy(g).wait()
                        w2_copy(g).wait()
                    for u in range(5, NT):
                        x_copy(u).wait()
                elif f == 4:
                    st_wo_ln2(3)
                    st_ln1(4)
                    st_qkv(4)
                    st_attn(4, 8, True)
            else:
                if f == 2 and t + 3 < NT:
                    st_wo_ln2(t + 3)
                if f == 3 and t + 4 < NT:
                    st_ln1(t + 4)
                    st_qkv(t + 4)
                    st_attn(t + 4, 8, True)
        pending = (t, acc)
    st_out(*pending)
    for s, part in enumerate(out_parts):
        out_copy(*part, s).wait()


@jax.jit
def pallas_adaLN_cond__sliding_local_dilated__dense_activation_relu__prompt_kernel(
        A_x, A_wqkv, A_wo, B_x, B_w1, B_w2, c, w_mod):
    del B_x
    hbm = pl.BlockSpec(memory_space=pltpu.HBM)
    outT = pl.pallas_call(
        _kernel,
        grid=(1,),
        in_specs=[hbm] * 7,
        out_specs=hbm,
        out_shape=jax.ShapeDtypeStruct((1, D, S), A_x.dtype),
        scratch_shapes=[
            pltpu.VMEM((D, S), bf16),
            pltpu.VMEM((D, S), bf16),
            pltpu.VMEM((1, D), bf16),
            pltpu.VMEM((D, 3 * D), bf16),
            pltpu.VMEM((5, DP, 128), f32),
            pltpu.VMEM((NQKV, DP), bf16),
            pltpu.VMEM((D, D), bf16),
            pltpu.VMEM((D, DP), bf16),
            pltpu.VMEM((D, F), bf16),
            pltpu.VMEM((D, F), bf16),
            pltpu.VMEM((D, 6 * D), bf16),
            pltpu.VMEM((6 * D, 128), f32),
            pltpu.VMEM((2, TM, DP), bf16),
            pltpu.VMEM((3, TM, DP), f32),
            pltpu.VMEM((5, HALO + S, 128), f32),
            pltpu.VMEM((5, HALO + S, 128), f32),
            pltpu.VMEM((3, TM, DP), bf16),
            pltpu.VMEM((S, D), bf16),
            pltpu.VMEM((4, D, TM), f32),
            pltpu.SemaphoreType.DMA((8,)),
            pltpu.SemaphoreType.DMA((NF,)),
            pltpu.SemaphoreType.DMA((NF,)),
            pltpu.SemaphoreType.DMA((NT,)),
            pltpu.SemaphoreType.DMA((NT - 1 + TM // 128,)),
            pltpu.SemaphoreType.REGULAR,
        ],
        compiler_params=pltpu.CompilerParams(
            vmem_limit_bytes=100 * 1024 * 1024,
            flags={"XLA_TPU_FORCE_LP_LLO_SCHEDULER": True},
        ),
        name="adaln_block",
    )(jnp.transpose(A_x, (0, 2, 1)), c, A_wqkv, A_wo, B_w1, jnp.transpose(B_w2), w_mod)
    return jnp.transpose(outT, (0, 2, 1))
```
